```python
import os as _os
_os.environ.setdefault('JAX_PLATFORMS', 'cpu')
import jax
import jax.numpy as jnp

def _softmax(x, axis=-1):
    return jax.nn.softmax(x, axis=axis)

def _gelu(x):
    return jax.nn.gelu(x, approximate=True)

def _silu(x):
    return jax.nn.silu(x)

def _sigmoid(x):
    return jax.nn.sigmoid(x)

def _layernorm(x, axis=-1, eps=1e-05):
    m = jnp.mean(x, axis=axis, keepdims=True)
    v = jnp.var(x, axis=axis, keepdims=True)
    return (x - m) / jnp.sqrt(v + eps)

def _scatter_add(tgt, idx, src, axis=0):
    return tgt.at[idx].add(src)

def _segment_sum(src, seg, n):
    return jax.ops.segment_sum(src, seg, n)

class _Rng:

    def __init__(self, key):
        self._k = key

    def _next(self):
        self._k, sub = jax.random.split(self._k)
        return sub

    def normal(self, shape):
        return jax.random.normal(self._next(), shape, dtype=jnp.bfloat16)

    def randint(self, lo, hi, shape):
        return jax.random.randint(self._next(), shape, lo, hi, dtype=jnp.int32)

    def uniform(self, shape, lo=0.0, hi=1.0):
        return jax.random.uniform(self._next(), shape, jnp.bfloat16, lo, hi)

    def permutation(self, n):
        return jax.random.permutation(self._next(), n)
kernel_name = 'sequential_preLN__linear_attn_block__mixer_gmlp__prompt'

def setup_inputs():
    _rng = _Rng(jax.random.key(int.from_bytes(__import__("os").urandom(4), "little")))
    _w = lambda a: (lambda t: t.astype(jnp.bfloat16) if jnp.issubdtype(t.dtype, jnp.floating) else t)(jnp.asarray(a))

    def _A_setup():
        B, S, D = (1, 2048, 512)
        return {'x': _w((lambda *s: _rng.normal(s) * 0.05)(B, S, D)), 'wqkv': _w((lambda *s: _rng.normal(s) * 0.05)(D, 3 * D)), 'wo': _w((lambda *s: _rng.normal(s) * 0.05)(D, D))}
    _A_in = _A_setup()

    def _B_setup():
        B, S, D, F = (1, 2048, 512, 1792)
        Fh = F // 2
        return {'x': _w((lambda *s: _rng.normal(s) * 0.05)(B, S, D)), 'w_in': _w((lambda *s: _rng.normal(s) * 0.4)(D, 2 * Fh)), 'w_sp': _w(0.01 * (lambda *s: _rng.normal(s) * 0.4)(S, S)), 'b_sp': _w(1.0 + 0.01 * (lambda *s: _rng.normal(s) * 0.05)(S)), 'w_out': _w((lambda *s: _rng.normal(s) * 0.05)(Fh, D))}
    _B_in = _B_setup()
    return {'A_x': _A_in['x'], 'A_wqkv': _A_in['wqkv'], 'A_wo': _A_in['wo'], 'B_x': _B_in['x'], 'B_w_in': _B_in['w_in'], 'B_w_sp': _B_in['w_sp'], 'B_b_sp': _B_in['b_sp'], 'B_w_out': _B_in['w_out']}

def reference(A_x, A_wqkv, A_wo, B_x, B_w_in, B_w_sp, B_b_sp, B_w_out):

    def _A_ref(x, wqkv, wo):
        B, S, D = x.shape
        H = 32
        Dh = D // H
        qkv = (lambda x, *d: x.transpose(*d))((x @ wqkv).reshape(B, S, 3, H, Dh), 2, 0, 3, 1, 4)
        q, k, v = (qkv[0], qkv[1], qkv[2])
        phi = lambda t: jnp.where(t > 0, t + 1, jnp.exp(t)) + 1e-06
        pq, pk = (phi(q), phi(k))
        kv = jnp.einsum('bhsd,bhse->bhde', pk, v)
        z = jnp.einsum('bhsd->bhd', pk)
        num = jnp.einsum('bhqd,bhde->bhqe', pq, kv)
        den = jnp.einsum('bhqd,bhd->bhq', pq, z)[..., None] + 1e-06
        o = num / den
        return (lambda x, *d: x.transpose(*d))(o, 0, 2, 1, 3).reshape(B, S, D) @ wo

    def _B_ref(x, w_in, w_sp, b_sp, w_out):
        B, S, D = x.shape
        F = w_in.shape[-1]
        Fh = F // 2
        z = _gelu(jnp.einsum('bsd,df->bsf', x, w_in))
        z1 = z[..., :Fh].copy()
        z2 = _layernorm(z[..., Fh:], axis=-1)
        g = jnp.einsum('ts,bsf->btf', w_sp, z2) + b_sp[None, :, None]
        return jnp.einsum('bsf,fd->bsd', z1 * g, w_out)
    x = A_x
    h = x + _A_ref(_layernorm(x, axis=-1), A_wqkv, A_wo)
    h2 = h + _B_ref(_layernorm(h, axis=-1), B_w_in, B_w_sp, B_b_sp, B_w_out)
    return h2
```

```python
import jax
import jax.numpy as jnp
from jax import lax
import jax.experimental.pallas as pl
import jax.experimental.pallas.tpu as pltpu

_LN_EPS = 1e-5
_PHI_EPS = 1e-6
_GELU_C = 0.7978845608028654
_LANES = 128


def _ln(x):
    m = jnp.mean(x, axis=-1, keepdims=True)
    xc = x - m
    v = jnp.mean(xc * xc, axis=-1, keepdims=True)
    return xc * lax.rsqrt(v + _LN_EPS)


def _phi(t):
    return jnp.where(t > 0, t + 1.0, jnp.exp(t)) + _PHI_EPS


def _gelu(x):
    inner = _GELU_C * (x + 0.044715 * (x * x * x))
    return 0.5 * x * (1.0 + jnp.tanh(inner))


def _dot(a, b):
    return jnp.dot(a, b, preferred_element_type=jnp.float32)


def _make_kernel(S, D, H, F, TM):
    DH = D // H
    FH = F // 2
    NB = S // TM
    NG = D // _LANES
    bf16 = jnp.bfloat16
    f32 = jnp.float32

    def kernel(x_hbm, wqkv_hbm, wo_hbm, win_hbm, wsp_hbm, bsp_hbm, wout_hbm,
               out_hbm,
               x_v, wqkv_v, wo_v, win_v, wsp_v, bsp_v, wout_v,
               pq_v, h_v, z1_v, z2_v, kv_acc, z_acc, kvz_v, bias_v, out_v,
               x_sem, w_sem, sp_sem, o_sem):
        def x_copy(i):
            return pltpu.make_async_copy(
                x_hbm.at[0, pl.ds(i * TM, TM), :], x_v.at[pl.ds(i * TM, TM), :],
                x_sem.at[i])

        def sp_copy(i):
            return pltpu.make_async_copy(
                wsp_hbm.at[pl.ds(i * TM, TM), :], wsp_v.at[pl.ds(i * TM, TM), :],
                sp_sem.at[i])

        def o_copy(i):
            return pltpu.make_async_copy(
                out_v.at[pl.ds(i * TM, TM), :], out_hbm.at[0, pl.ds(i * TM, TM), :],
                o_sem.at[i])

        w_copies = [
            pltpu.make_async_copy(wqkv_hbm, wqkv_v, w_sem.at[0]),
            pltpu.make_async_copy(wo_hbm, wo_v, w_sem.at[1]),
            pltpu.make_async_copy(win_hbm, win_v, w_sem.at[2]),
            pltpu.make_async_copy(wout_hbm, wout_v, w_sem.at[3]),
            pltpu.make_async_copy(bsp_hbm, bsp_v, w_sem.at[4]),
        ]

        x_copy(0).start()
        w_copies[0].start()
        for i in range(1, NB):
            x_copy(i).start()
        for c in w_copies[1:]:
            c.start()
        for i in range(NB):
            sp_copy(i).start()

        kv_acc[...] = jnp.zeros_like(kv_acc)
        z_acc[...] = jnp.zeros_like(z_acc)
        w_copies[0].wait()

        def phase1(i, carry):
            r = pl.multiple_of(i * TM, TM)
            x_copy(i).wait()
            xn = _ln(x_v[pl.ds(r, TM), :].astype(f32)).astype(bf16)
            q = _dot(xn, wqkv_v[:, 0:D])
            pq_v[pl.ds(r, TM), :] = _phi(q).astype(bf16)
            pk = _phi(_dot(xn, wqkv_v[:, D:2 * D]))
            z_acc[...] += jnp.sum(pk, axis=0, keepdims=True)
            pk = pk.astype(bf16)
            v = _dot(xn, wqkv_v[:, 2 * D:3 * D]).astype(bf16)
            for g in range(NG):
                sl = slice(g * _LANES, (g + 1) * _LANES)
                kv_acc[g] += lax.dot_general(
                    pk[:, sl], v[:, sl], (((0,), (0,)), ((), ())),
                    preferred_element_type=f32)
            return carry

        lax.fori_loop(0, NB, phase1, 0)

        row_h = lax.broadcasted_iota(jnp.int32, (_LANES, _LANES), 0) // DH
        col_h = lax.broadcasted_iota(jnp.int32, (_LANES, _LANES), 1) // DH
        mask = row_h == col_h
        for g in range(NG):
            sl = slice(g * _LANES, (g + 1) * _LANES)
            kvz_v[g, :, 0:_LANES] = jnp.where(mask, kv_acc[g], 0.0).astype(bf16)
            zb = jnp.broadcast_to(z_acc[:, sl], (_LANES, _LANES)).T
            kvz_v[g, :, _LANES:2 * _LANES] = jnp.where(mask, zb, 0.0).astype(bf16)

        w_copies[4].wait()
        for c in range(S // _LANES):
            brow = bsp_v[c:c + 1, :].astype(f32)
            bias_v[c * _LANES:(c + 1) * _LANES, :] = jnp.broadcast_to(
                brow, (_LANES, _LANES)).T

        w_copies[1].wait()
        w_copies[2].wait()

        def phase2(i, carry):
            r = pl.multiple_of(i * TM, TM)
            os_ = []
            for g in range(NG):
                sl = slice(g * _LANES, (g + 1) * _LANES)
                nd = _dot(pq_v[pl.ds(r, TM), sl], kvz_v[g])
                os_.append((nd[:, :_LANES] / (nd[:, _LANES:] + _PHI_EPS)).astype(bf16))
            o = jnp.concatenate(os_, axis=-1)
            h = x_v[pl.ds(r, TM), :].astype(f32) + _dot(o, wo_v[...])
            h_v[pl.ds(r, TM), :] = h
            hn = _ln(h).astype(bf16)
            z1_v[pl.ds(r, TM), :] = _gelu(_dot(hn, win_v[:, 0:FH])).astype(bf16)
            z2_v[pl.ds(r, TM), :] = _ln(_gelu(_dot(hn, win_v[:, FH:F]))).astype(bf16)
            return carry

        lax.fori_loop(0, NB, phase2, 0)

        w_copies[3].wait()

        def phase3(i, carry):
            r = pl.multiple_of(i * TM, TM)
            sp_copy(i).wait()
            g = _dot(wsp_v[pl.ds(r, TM), :], z2_v[...])
            b = bias_v[pl.ds(r, TM), :]
            g = g + jnp.concatenate([b] * (FH // _LANES), axis=-1)
            t = (z1_v[pl.ds(r, TM), :].astype(f32) * g).astype(bf16)
            y = h_v[pl.ds(r, TM), :] + _dot(t, wout_v[...])
            out_v[pl.ds(r, TM), :] = y.astype(out_v.dtype)
            o_copy(i).start()
            return carry

        lax.fori_loop(0, NB, phase3, 0)
        for i in range(NB):
            o_copy(i).wait()

    scratch = [
        pltpu.VMEM((S, D), bf16),
        pltpu.VMEM((D, 3 * D), bf16),
        pltpu.VMEM((D, D), bf16),
        pltpu.VMEM((D, F), bf16),
        pltpu.VMEM((S, S), bf16),
        pltpu.VMEM((S // _LANES, _LANES), bf16),
        pltpu.VMEM((FH, D), bf16),
        pltpu.VMEM((S, D), bf16),
        pltpu.VMEM((S, D), f32),
        pltpu.VMEM((S, FH), bf16),
        pltpu.VMEM((S, FH), bf16),
        pltpu.VMEM((NG, _LANES, _LANES), f32),
        pltpu.VMEM((1, D), f32),
        pltpu.VMEM((NG, _LANES, 2 * _LANES), bf16),
        pltpu.VMEM((S, _LANES), f32),
        pltpu.VMEM((S, D), bf16),
        pltpu.SemaphoreType.DMA((NB,)),
        pltpu.SemaphoreType.DMA((5,)),
        pltpu.SemaphoreType.DMA((NB,)),
        pltpu.SemaphoreType.DMA((NB,)),
    ]
    return kernel, scratch


@jax.jit
def pallas_sequential_preLN__linear_attn_block__mixer_gmlp__prompt_kernel(
    A_x: jax.Array,
    A_wqkv: jax.Array,
    A_wo: jax.Array,
    B_x: jax.Array,
    B_w_in: jax.Array,
    B_w_sp: jax.Array,
    B_b_sp: jax.Array,
    B_w_out: jax.Array,
):
    del B_x
    B, S, D = A_x.shape
    assert B == 1
    F = B_w_in.shape[-1]
    H = 32
    TM = 512
    kernel, scratch = _make_kernel(S, D, H, F, TM)
    any_spec = pl.BlockSpec(memory_space=pl.ANY)
    return pl.pallas_call(
        kernel,
        out_shape=jax.ShapeDtypeStruct((B, S, D), A_x.dtype),
        in_specs=[any_spec] * 7,
        out_specs=any_spec,
        scratch_shapes=scratch,
        compiler_params=pltpu.CompilerParams(vmem_limit_bytes=100 * 1024 * 1024),
    )(A_x, A_wqkv, A_wo, B_w_in, B_w_sp, B_b_sp.reshape(S // _LANES, _LANES),
      B_w_out)
```

```python
import jax
import jax.numpy as jnp
from jax import lax
import jax.experimental.pallas as pl
import jax.experimental.pallas.tpu as pltpu

_LN_EPS = 1e-5
_PHI_EPS = 1e-6
_GELU_C = 0.7978845608028654
_LANES = 128


def _ln(x):
    m = jnp.mean(x, axis=-1, keepdims=True)
    xc = x - m
    v = jnp.mean(xc * xc, axis=-1, keepdims=True)
    return xc * lax.rsqrt(v + _LN_EPS)


def _phi(t):
    return jnp.where(t > 0, t + 1.0, jnp.exp(t)) + _PHI_EPS


def _gelu2(x):
    p = (x * x) * (_GELU_C * 0.044715) + _GELU_C
    return x * jnp.tanh(x * p) + x


def _ln_half(w):
    m = jnp.mean(w, axis=-1, keepdims=True)
    wc = w - m
    v = jnp.mean(wc * wc, axis=-1, keepdims=True)
    return wc * (0.5 * lax.rsqrt(v + 4.0 * _LN_EPS))


def _dot(a, b):
    return jnp.dot(a, b, preferred_element_type=jnp.float32)


def _make_kernel(S, D, H, F, TM):
    DH = D // H
    FH = F // 2
    NB = S // TM
    NG = D // _LANES
    bf16 = jnp.bfloat16
    f32 = jnp.float32

    def kernel(x_hbm, wqkv_hbm, wo_hbm, win_hbm, wsp_hbm, bsp_hbm, wout_hbm,
               out_hbm,
               x_v, wqkv_v, wo_v, win_v, wsp_v, bsp_v, wout_v,
               pq_v, h_v, z1_v, z2_v, kv_acc, z_acc, zm_v, m_v, g_v, out_v, bias_v, xn_v,
               x_sem, w_sem, sp_sem, o_sem):
        def x_copy(i):
            return pltpu.make_async_copy(
                x_hbm.at[0, pl.ds(i * TM, TM), :], x_v.at[pl.ds(i * TM, TM), :],
                x_sem.at[i])

        def sp_copy(i):
            return pltpu.make_async_copy(
                wsp_hbm.at[:, pl.ds(i * TM, TM)], wsp_v.at[i], sp_sem.at[i])

        def o_copy(i):
            return pltpu.make_async_copy(
                out_v.at[pl.ds(i * TM, TM), :], out_hbm.at[0, pl.ds(i * TM, TM), :],
                o_sem.at[i])

        qkv_copies = [
            pltpu.make_async_copy(wqkv_hbm.at[:, pl.ds(j * D, D)],
                                  wqkv_v.at[:, pl.ds(j * D, D)], w_sem.at[5 + j])
            for j in range(3)]
        w_copies = [
            None,
            pltpu.make_async_copy(wo_hbm, wo_v, w_sem.at[1]),
            pltpu.make_async_copy(win_hbm, win_v, w_sem.at[2]),
            pltpu.make_async_copy(wout_hbm, wout_v, w_sem.at[3]),
            pltpu.make_async_copy(bsp_hbm, bsp_v, w_sem.at[4]),
        ]

        def ln_x(r):
            return _ln(x_v[pl.ds(r, TM), :].astype(f32)).astype(bf16)

        w_copies[4].start()
        x_copy(0).start()
        qkv_copies[2].start()

        kv_acc[...] = jnp.zeros_like(kv_acc)
        z_acc[...] = jnp.zeros_like(z_acc)

        w_copies[4].wait()
        qkv_copies[1].start()
        qkv_copies[0].start()
        x_copy(1).start()
        for c in range(S // _LANES):
            brow = bsp_v[c:c + 1, :].astype(f32) * 0.5
            bias_v[c * _LANES:(c + 1) * _LANES, :] = jnp.broadcast_to(
                brow, (_LANES, _LANES)).T

        x_copy(0).wait()
        xn_v[0:TM, :] = ln_x(0)

        def qproj(r):
            q = _dot(xn_v[pl.ds(r, TM), :], wqkv_v[:, 0:D])
            pq_v[pl.ds(r, TM), :] = _phi(q).astype(bf16)

        def phase1_body(r, r_next, first):
            xn = xn_v[pl.ds(r, TM), :]

            def vdot():
                return _dot(xn, wqkv_v[:, 2 * D:3 * D]).astype(bf16)

            if first:
                qkv_copies[2].wait()
                v = vdot()
                qkv_copies[1].wait()
                qkv_copies[0].wait()
                x_copy(1).wait()
                for i in range(2, NB):
                    x_copy(i).start()
                for c in w_copies[1:3]:
                    c.start()
                sp_copy(0).start()
            pk = _phi(_dot(xn, wqkv_v[:, D:2 * D]))
            z_acc[...] += jnp.sum(pk, axis=0, keepdims=True)
            pk = pk.astype(bf16)
            if first:
                qproj(r)
            else:
                v = vdot()
            for g in range(NG):
                sl = slice(g * _LANES, (g + 1) * _LANES)
                kv_acc[g] += lax.dot_general(
                    pk[:, sl], v[:, sl], (((0,), (0,)), ((), ())),
                    preferred_element_type=f32)
            xn_v[pl.ds(r_next, TM), :] = ln_x(r_next)

        phase1_body(0, TM, True)

        def phase1(i, carry):
            r = pl.multiple_of(i * TM, TM)
            nxt = jnp.minimum(i + 1, NB - 1)

            @pl.when(i + 1 < NB)
            def _():
                x_copy(i + 1).wait()

            phase1_body(r, pl.multiple_of(nxt * TM, TM), False)
            return carry

        lax.fori_loop(1, NB, phase1, 0)

        w_copies[1].wait()
        row_h = lax.broadcasted_iota(jnp.int32, (_LANES, _LANES), 0) // DH
        col_h = lax.broadcasted_iota(jnp.int32, (_LANES, _LANES), 1) // DH
        mask = row_h == col_h
        for g in range(NG):
            sl = slice(g * _LANES, (g + 1) * _LANES)
            kvm = jnp.where(mask, kv_acc[g], 0.0).astype(bf16)
            m_v[sl, :] = _dot(kvm, wo_v[sl, :]).astype(bf16)
            zb = jnp.broadcast_to(z_acc[:, sl], (_LANES, _LANES)).T
            zm_v[g] = jnp.where(mask, zb, 0.0).astype(bf16)

        w_copies[2].wait()
        for i in range(1, NB):
            sp_copy(i).start()
        w_copies[3].start()

        def ab(r, fill):
            os_ = []
            for g in range(NG):
                sl = slice(g * _LANES, (g + 1) * _LANES)
                pq = pq_v[pl.ds(r, TM), sl]
                den = _dot(pq, zm_v[g]) + _PHI_EPS
                rc = pl.reciprocal(den, approx=True)
                rc = rc * (2.0 - den * rc)
                os_.append((pq.astype(f32) * rc).astype(bf16))
            o = jnp.concatenate(os_, axis=-1)
            fill(0)
            h = x_v[pl.ds(r, TM), :].astype(f32) + _dot(o, m_v[...])
            h_v[pl.ds(r, TM), :] = h
            hn = _ln(h).astype(bf16)
            fill(1)
            z2_v[pl.ds(r, TM), :] = _ln_half(_gelu2(_dot(hn, win_v[:, FH:F]))).astype(bf16)
            fill(2)
            z1_v[pl.ds(r, TM), :] = _gelu2(_dot(hn, win_v[:, 0:FH])).astype(bf16)
            fill(3)

        def fill0(j):
            if j + 1 < NB:
                qproj((j + 1) * TM)

        ab(0, fill0)

        def phase2(i, carry):
            k = i - 1
            sp_copy(k).wait()
            z2p = z2_v[pl.ds(pl.multiple_of(k * TM, TM), TM), :]

            def fill(j):
                rows = slice(j * TM, (j + 1) * TM)
                prev = jnp.where(k == 0, 0.0, g_v[rows, :])
                g_v[rows, :] = prev + _dot(wsp_v[k, rows, :], z2p)

            ab(pl.multiple_of(i * TM, TM), fill)
            return carry

        lax.fori_loop(1, NB, phase2, 0)

        w_copies[3].wait()
        sp_copy(NB - 1).wait()

        def phase3(i, carry):
            r = pl.multiple_of(i * TM, TM)
            b = bias_v[pl.ds(r, TM), :]
            g = g_v[pl.ds(r, TM), :] + jnp.concatenate([b] * (FH // _LANES), axis=-1)
            g = g + _dot(wsp_v[NB - 1, pl.ds(r, TM), :], z2_v[(NB - 1) * TM:NB * TM, :])
            t = (z1_v[pl.ds(r, TM), :].astype(f32) * g).astype(bf16)
            y = h_v[pl.ds(r, TM), :] + _dot(t, wout_v[...])
            out_v[pl.ds(r, TM), :] = y.astype(out_v.dtype)
            o_copy(i).start()
            return carry

        lax.fori_loop(0, NB, phase3, 0)
        for i in range(NB):
            o_copy(i).wait()

    scratch = [
        pltpu.VMEM((S, D), bf16),
        pltpu.VMEM((D, 3 * D), bf16),
        pltpu.VMEM((D, D), bf16),
        pltpu.VMEM((D, F), bf16),
        pltpu.VMEM((NB, S, TM), bf16),
        pltpu.VMEM((S // _LANES, _LANES), bf16),
        pltpu.VMEM((FH, D), bf16),
        pltpu.VMEM((S, D), bf16),
        pltpu.VMEM((S, D), f32),
        pltpu.VMEM((S, FH), bf16),
        pltpu.VMEM((S, FH), bf16),
        pltpu.VMEM((NG, _LANES, _LANES), f32),
        pltpu.VMEM((1, D), f32),
        pltpu.VMEM((NG, _LANES, _LANES), bf16),
        pltpu.VMEM((D, D), bf16),
        pltpu.VMEM((S, FH), f32),
        pltpu.VMEM((S, D), bf16),
        pltpu.VMEM((S, _LANES), f32),
        pltpu.VMEM((S, D), bf16),
        pltpu.SemaphoreType.DMA((NB,)),
        pltpu.SemaphoreType.DMA((8,)),
        pltpu.SemaphoreType.DMA((NB,)),
        pltpu.SemaphoreType.DMA((NB,)),
    ]
    return kernel, scratch


@jax.jit
def pallas_sequential_preLN__linear_attn_block__mixer_gmlp__prompt_kernel(
    A_x: jax.Array,
    A_wqkv: jax.Array,
    A_wo: jax.Array,
    B_x: jax.Array,
    B_w_in: jax.Array,
    B_w_sp: jax.Array,
    B_b_sp: jax.Array,
    B_w_out: jax.Array,
):
    del B_x
    B, S, D = A_x.shape
    assert B == 1
    F = B_w_in.shape[-1]
    H = 32
    TM = 512
    kernel, scratch = _make_kernel(S, D, H, F, TM)
    any_spec = pl.BlockSpec(memory_space=pl.ANY)
    return pl.pallas_call(
        kernel,
        out_shape=jax.ShapeDtypeStruct((B, S, D), A_x.dtype),
        in_specs=[any_spec] * 7,
        out_specs=any_spec,
        scratch_shapes=scratch,
        compiler_params=pltpu.CompilerParams(vmem_limit_bytes=100 * 1024 * 1024),
    )(A_x, A_wqkv, A_wo, B_w_in, B_w_sp, B_b_sp.reshape(S // _LANES, _LANES),
      B_w_out)
```

```python
import jax
import jax.numpy as jnp
from jax import lax
import jax.experimental.pallas as pl
import jax.experimental.pallas.tpu as pltpu

_LN_EPS = 1e-5
_PHI_EPS = 1e-6
_GELU_C = 0.7978845608028654
_LANES = 128


def _ln(x):
    m = jnp.mean(x, axis=-1, keepdims=True)
    xc = x - m
    v = jnp.mean(xc * xc, axis=-1, keepdims=True)
    return xc * lax.rsqrt(v + _LN_EPS)


def _phi(t):
    return jnp.where(t > 0, t + 1.0, jnp.exp(t)) + _PHI_EPS


def _gelu2(x):
    p = (x * x) * (_GELU_C * 0.044715) + _GELU_C
    return x * jnp.tanh(x * p) + x


def _ln_half(w):
    m = jnp.mean(w, axis=-1, keepdims=True)
    wc = w - m
    v = jnp.mean(wc * wc, axis=-1, keepdims=True)
    return wc * (0.5 * lax.rsqrt(v + 4.0 * _LN_EPS))


def _dot(a, b):
    return jnp.dot(a, b, preferred_element_type=jnp.float32)


def _make_kernel(S, D, H, F, TM):
    DH = D // H
    FH = F // 2
    NB = S // TM
    NG = D // _LANES
    OC = _LANES
    NOC = D // OC
    assert NB == 4 and S % TM == 0 and D % _LANES == 0 and FH % _LANES == 0
    assert _LANES % DH == 0
    bf16 = jnp.bfloat16
    f32 = jnp.float32

    def kernel(x_hbm, wqkv_hbm, wo_hbm, win_hbm, wsp_hbm, bsp_hbm, wout_hbm,
               out_hbm,
               x_v, wqkv_v, wo_v, win_v, wsp_v, bsp_v, wout_v,
               pq_v, h_v, z1_v, z2_v, kv_acc, z_acc, zm_v, m_v, g_v, out_v,
               bias_v, xn_v,
               x_sem, w_sem, sp_sem, o_sem):
        def x_copy(i):
            return pltpu.make_async_copy(
                x_hbm.at[0, pl.ds(i * TM, TM), :], x_v.at[pl.ds(i * TM, TM), :],
                x_sem.at[i])

        def sp_copy(i):
            return pltpu.make_async_copy(
                wsp_hbm.at[:, pl.ds(i * TM, TM)], wsp_v.at[i], sp_sem.at[i])

        def o_copy(i, j):
            cols = pl.ds(j * OC, OC)
            return pltpu.make_async_copy(
                out_v.at[pl.ds(i * TM, TM), cols],
                out_hbm.at[0, pl.ds(i * TM, TM), cols],
                o_sem.at[i * NOC + j])

        wq_copy, wk_copy, wv_copy = [
            pltpu.make_async_copy(wqkv_hbm.at[:, pl.ds(j * D, D)],
                                  wqkv_v.at[:, pl.ds(j * D, D)], w_sem.at[j])
            for j in range(3)]
        wo_copy = pltpu.make_async_copy(wo_hbm, wo_v, w_sem.at[3])
        win_copy = pltpu.make_async_copy(win_hbm, win_v, w_sem.at[4])
        wout_copy = pltpu.make_async_copy(wout_hbm, wout_v, w_sem.at[5])
        bsp_copy = pltpu.make_async_copy(bsp_hbm, bsp_v, w_sem.at[6])

        def ln_x(r):
            return _ln(x_v[pl.ds(r, TM), :].astype(f32)).astype(bf16)

        bsp_copy.start()
        x_copy(0).start()
        wv_copy.start()

        kv_acc[...] = jnp.zeros_like(kv_acc)
        z_acc[...] = jnp.zeros_like(z_acc)

        bsp_copy.wait()
        for c in range(S // _LANES):
            brow = bsp_v[c:c + 1, :].astype(f32) * 0.5
            bias_v[c * _LANES:(c + 1) * _LANES, :] = jnp.broadcast_to(
                brow, (_LANES, _LANES)).T

        x_copy(0).wait()
        wk_copy.start()
        x_copy(1).start()
        xn_v[0:TM, :] = ln_x(0)

        def qproj(r):
            q = _dot(xn_v[pl.ds(r, TM), :], wqkv_v[:, 0:D])
            pq_v[pl.ds(r, TM), :] = _phi(q).astype(bf16)

        def phase1_block(r, r_next, first):
            xn = xn_v[pl.ds(r, TM), :]

            def vdot():
                return _dot(xn, wqkv_v[:, 2 * D:3 * D]).astype(bf16)

            if first:
                wv_copy.wait()
                v = vdot()
                wk_copy.wait()
                x_copy(1).wait()
                for i in range(2, NB):
                    x_copy(i).start()
                wq_copy.start()
                wo_copy.start()
                win_copy.start()
                sp_copy(0).start()
            pk = _phi(_dot(xn, wqkv_v[:, D:2 * D]))
            z_acc[...] += jnp.sum(pk, axis=0, keepdims=True)
            pk = pk.astype(bf16)
            if not first:
                v = vdot()
            for g in range(NG):
                sl = slice(g * _LANES, (g + 1) * _LANES)
                kv_acc[g] += lax.dot_general(
                    pk[:, sl], v[:, sl], (((0,), (0,)), ((), ())),
                    preferred_element_type=f32)
            if r_next is not None:
                xn_v[pl.ds(r_next, TM), :] = ln_x(r_next)

        phase1_block(0, TM, True)
        for i in range(1, NB):
            if i + 1 < NB:
                x_copy(i + 1).wait()
                phase1_block(i * TM, (i + 1) * TM, False)
            else:
                phase1_block(i * TM, None, False)

        wo_copy.wait()
        wq_copy.wait()
        win_copy.wait()
        for i in range(1, NB):
            sp_copy(i).start()
        wout_copy.start()

        qproj(0)
        row_h = lax.broadcasted_iota(jnp.int32, (_LANES, _LANES), 0) // DH
        col_h = lax.broadcasted_iota(jnp.int32, (_LANES, _LANES), 1) // DH
        mask = row_h == col_h
        for g in range(NG):
            sl = slice(g * _LANES, (g + 1) * _LANES)
            kvm = jnp.where(mask, kv_acc[g], 0.0).astype(bf16)
            m_v[sl, :] = _dot(kvm, wo_v[sl, :]).astype(bf16)
            zb = jnp.broadcast_to(z_acc[:, sl], (_LANES, _LANES)).T
            zm_v[g] = jnp.where(mask, zb, 0.0).astype(bf16)

        def block2(r, fill):
            os_ = []
            for g in range(NG):
                sl = slice(g * _LANES, (g + 1) * _LANES)
                pq = pq_v[pl.ds(r, TM), sl]
                den = _dot(pq, zm_v[g]) + _PHI_EPS
                rc = pl.reciprocal(den, approx=True)
                rc = rc * (2.0 - den * rc)
                os_.append((pq.astype(f32) * rc).astype(bf16))
            o = jnp.concatenate(os_, axis=-1)
            fill(0)
            h = x_v[pl.ds(r, TM), :].astype(f32) + _dot(o, m_v[...])
            h_v[pl.ds(r, TM), :] = h
            hn = _ln(h).astype(bf16)
            fill(1)
            z2_v[pl.ds(r, TM), :] = _ln_half(
                _gelu2(_dot(hn, win_v[:, FH:F]))).astype(bf16)
            fill(2)
            z1_v[pl.ds(r, TM), :] = _gelu2(_dot(hn, win_v[:, 0:FH])).astype(bf16)
            fill(3)

        def fill_q(j):
            if j + 2 < NB:
                qproj((j + 2) * TM)

        qproj(TM)
        block2(0, fill_q)

        def phase2(i, carry):
            k = i - 1
            sp_copy(k).wait()
            z2p = z2_v[pl.ds(pl.multiple_of(k * TM, TM), TM), :]

            def fill_g(j):
                rows = slice(j * TM, (j + 1) * TM)
                prev = jnp.where(k == 0, 0.0, g_v[rows, :])
                g_v[rows, :] = prev + _dot(wsp_v[k, rows, :], z2p)

            block2(pl.multiple_of(i * TM, TM), fill_g)
            return carry

        lax.fori_loop(1, NB, phase2, 0)

        wout_copy.wait()
        sp_copy(NB - 1).wait()

        def phase3(i, carry):
            r = pl.multiple_of(i * TM, TM)
            b = bias_v[pl.ds(r, TM), :]
            g = g_v[pl.ds(r, TM), :] + jnp.concatenate([b] * (FH // _LANES), axis=-1)
            g = g + _dot(wsp_v[NB - 1, pl.ds(r, TM), :],
                         z2_v[(NB - 1) * TM:NB * TM, :])
            t = (z1_v[pl.ds(r, TM), :].astype(f32) * g).astype(bf16)
            for j in range(NOC):
                cs = slice(j * OC, (j + 1) * OC)
                y = h_v[pl.ds(r, TM), cs] + _dot(t, wout_v[:, cs])
                out_v[pl.ds(r, TM), cs] = y.astype(out_v.dtype)
                o_copy(i, j).start()
            return carry

        lax.fori_loop(0, NB, phase3, 0)
        for i in range(NB):
            for j in range(NOC):
                o_copy(i, j).wait()

    scratch = [
        pltpu.VMEM((S, D), bf16),
        pltpu.VMEM((D, 3 * D), bf16),
        pltpu.VMEM((D, D), bf16),
        pltpu.VMEM((D, F), bf16),
        pltpu.VMEM((NB, S, TM), bf16),
        pltpu.VMEM((S // _LANES, _LANES), bf16),
        pltpu.VMEM((FH, D), bf16),
        pltpu.VMEM((S, D), bf16),
        pltpu.VMEM((S, D), f32),
        pltpu.VMEM((S, FH), bf16),
        pltpu.VMEM((S, FH), bf16),
        pltpu.VMEM((NG, _LANES, _LANES), f32),
        pltpu.VMEM((1, D), f32),
        pltpu.VMEM((NG, _LANES, _LANES), bf16),
        pltpu.VMEM((D, D), bf16),
        pltpu.VMEM((S, FH), f32),
        pltpu.VMEM((S, D), bf16),
        pltpu.VMEM((S, _LANES), f32),
        pltpu.VMEM((S, D), bf16),
        pltpu.SemaphoreType.DMA((NB,)),
        pltpu.SemaphoreType.DMA((7,)),
        pltpu.SemaphoreType.DMA((NB,)),
        pltpu.SemaphoreType.DMA((NB * NOC,)),
    ]
    return kernel, scratch


@jax.jit
def pallas_sequential_preLN__linear_attn_block__mixer_gmlp__prompt_kernel(
    A_x: jax.Array,
    A_wqkv: jax.Array,
    A_wo: jax.Array,
    B_x: jax.Array,
    B_w_in: jax.Array,
    B_w_sp: jax.Array,
    B_b_sp: jax.Array,
    B_w_out: jax.Array,
):
    del B_x
    B, S, D = A_x.shape
    assert B == 1
    F = B_w_in.shape[-1]
    H = 32
    TM = 512
    kernel, scratch = _make_kernel(S, D, H, F, TM)
    any_spec = pl.BlockSpec(memory_space=pl.ANY)
    return pl.pallas_call(
        kernel,
        out_shape=jax.ShapeDtypeStruct((B, S, D), A_x.dtype),
        in_specs=[any_spec] * 7,
        out_specs=any_spec,
        scratch_shapes=scratch,
        compiler_params=pltpu.CompilerParams(vmem_limit_bytes=100 * 1024 * 1024),
    )(A_x, A_wqkv, A_wo, B_w_in, B_w_sp, B_b_sp.reshape(S // _LANES, _LANES),
      B_w_out)
```
